```python
import os as _os
_os.environ.setdefault("JAX_PLATFORMS", "cpu")
import jax
import jax.numpy as jnp

def _softmax(x, axis=-1):
    return jax.nn.softmax(x, axis=axis)
def _gelu(x):
    return jax.nn.gelu(x, approximate=True)
def _silu(x):
    return jax.nn.silu(x)
def _sigmoid(x):
    return jax.nn.sigmoid(x)
def _layernorm(x, axis=-1, eps=1e-5):
    m = jnp.mean(x, axis=axis, keepdims=True)
    v = jnp.var(x, axis=axis, keepdims=True)
    return (x - m) / jnp.sqrt(v + eps)
def _scatter_add(tgt, idx, src, axis=0):
    return tgt.at[idx].add(src)
def _segment_sum(src, seg, n):
    return jax.ops.segment_sum(src, seg, n)
class _Rng:
    def __init__(self, key):
        self._k = key
    def _next(self):
        self._k, sub = jax.random.split(self._k)
        return sub
    def normal(self, shape):
        return jax.random.normal(self._next(), shape, dtype=jnp.bfloat16)
    def randint(self, lo, hi, shape):
        return jax.random.randint(self._next(), shape, lo, hi, dtype=jnp.int32)
    def uniform(self, shape, lo=0.0, hi=1.0):
        return jax.random.uniform(self._next(), shape, jnp.bfloat16, lo, hi)
    def permutation(self, n):
        return jax.random.permutation(self._next(), n)


kernel_name = 'standalone__instancenorm__sampling'

def setup_inputs():
    _rng = _Rng(jax.random.key(int.from_bytes(__import__("os").urandom(4), "little")))
    _w = (lambda a: (lambda t: t.astype(jnp.bfloat16) if jnp.issubdtype(t.dtype, jnp.floating) else t)(jnp.asarray(a)))
    B, C, H, W = 16, 640, 16, 32
    return {
        "x": _w((lambda *s: _rng.normal(s) * 0.05)(B, C, H, W)),
        "g": _w((lambda *s: _rng.normal(s) * 0.05)(C) + 1.0),
        "b": _w((lambda *s: _rng.normal(s) * 0.05)(C)),
    }

def reference(x, g, b):
    mu = x.mean(axis=(-2, -1), keepdims=True)
    var = ((x - mu) * (x - mu)).mean(axis=(-2, -1), keepdims=True)
    xhat = (x - mu) / jnp.sqrt(var + 1e-5)
    return xhat * g.reshape(1, -1, 1, 1) + b.reshape(1, -1, 1, 1)
```

```python
import jax
import jax.numpy as jnp
import jax.experimental.pallas as pl
import jax.experimental.pallas.tpu as pltpu

_EPS = 1e-5


def _make_kernel(nb, hw, split, tail):
    rows = nb * hw
    row_bounds = (0, split * hw, rows - tail, rows)
    tail_slab = (rows - tail) // hw

    def kernel(x_hbm, g_hbm, b_hbm, o_hbm, buf, gbuf, bbuf, rsem, wsem, gsem):
        def read(k):
            lo, n = row_bounds[k], row_bounds[k + 1] - row_bounds[k]
            return pltpu.make_async_copy(
                x_hbm.at[pl.ds(lo, n)], buf.at[pl.ds(lo, n)], rsem.at[k])

        def write(k):
            lo, n = ((0, split * hw), (split * hw, rows - split * hw))[k]
            return pltpu.make_async_copy(
                buf.at[pl.ds(lo, n)], o_hbm.at[pl.ds(lo, n)], wsem.at[k])

        g_copy = pltpu.make_async_copy(g_hbm, gbuf, gsem.at[0])
        b_copy = pltpu.make_async_copy(b_hbm, bbuf, gsem.at[1])

        read(0).start()
        g_copy.start()
        b_copy.start()

        def slab(i, carry):
            @pl.when(i == 0)
            def _():
                read(1).start()
                read(2).start()
                g_copy.wait()
                b_copy.wait()
                read(0).wait()

            @pl.when(i == split)
            def _():
                read(1).wait()
                write(0).start()

            @pl.when(i == tail_slab)
            def _():
                read(2).wait()

            g = gbuf[...].astype(jnp.float32).reshape(1, -1)
            b = bbuf[...].astype(jnp.float32).reshape(1, -1)
            r0 = pl.multiple_of(i * hw, hw)
            x = buf[pl.ds(r0, hw), :].astype(jnp.float32)
            mu = jnp.sum(x, axis=0, keepdims=True) * (1.0 / hw)
            xc = x - mu
            var = jnp.sum(xc * xc, axis=0, keepdims=True) * (1.0 / hw)
            scale = jax.lax.rsqrt(var + _EPS) * g
            buf[pl.ds(r0, hw), :] = (xc * scale + b).astype(buf.dtype)
            return carry

        jax.lax.fori_loop(0, nb, slab, 0)
        write(1).start()
        write(0).wait()
        write(1).wait()

    return kernel


@jax.jit
def pallas_standalone__instancenorm__sampling_kernel(
    x: jax.Array,
    g: jax.Array,
    b: jax.Array,
):
    B, C, H, W = x.shape
    hw = H * W
    split = B // 2
    tail = hw // 2
    assert B >= 2 and hw % 32 == 0 and C % 128 == 0

    xt = jnp.transpose(x, (0, 2, 3, 1)).reshape(B * hw, C)
    out = pl.pallas_call(
        _make_kernel(B, hw, split, tail),
        in_specs=[pl.BlockSpec(memory_space=pl.ANY)] * 3,
        out_specs=pl.BlockSpec(memory_space=pl.ANY),
        out_shape=jax.ShapeDtypeStruct((B * hw, C), x.dtype),
        scratch_shapes=[
            pltpu.VMEM((B * hw, C), x.dtype),
            pltpu.VMEM((C,), g.dtype),
            pltpu.VMEM((C,), b.dtype),
            pltpu.SemaphoreType.DMA((3,)),
            pltpu.SemaphoreType.DMA((2,)),
            pltpu.SemaphoreType.DMA((2,)),
        ],
        compiler_params=pltpu.CompilerParams(vmem_limit_bytes=64 * 1024 * 1024),
    )(xt, g, b)
    return jnp.transpose(out.reshape(B, H, W, C), (0, 3, 1, 2))
```
